```python
import jax
import jax.numpy as jnp

def _softmax(x, axis=-1):
    return jax.nn.softmax(x, axis=axis)
def _gelu(x):
    return jax.nn.gelu(x, approximate=True)
def _silu(x):
    return jax.nn.silu(x)
def _sigmoid(x):
    return jax.nn.sigmoid(x)
def _layernorm(x, axis=-1, eps=1e-5):
    m = jnp.mean(x, axis=axis, keepdims=True)
    v = jnp.var(x, axis=axis, keepdims=True)
    return (x - m) / jnp.sqrt(v + eps)
def _scatter_add(tgt, idx, src, axis=0):
    return tgt.at[idx].add(src)
def _segment_sum(src, seg, n):
    return jax.ops.segment_sum(src, seg, n)
class _Rng:
    def __init__(self, key):
        self._k = key
    def _next(self):
        self._k, sub = jax.random.split(self._k)
        return sub
    def normal(self, shape):
        return jax.random.normal(self._next(), shape, dtype=jnp.bfloat16)
    def randint(self, lo, hi, shape):
        return jax.random.randint(self._next(), shape, lo, hi, dtype=jnp.int32)
    def uniform(self, shape, lo=0.0, hi=1.0):
        return jax.random.uniform(self._next(), shape, jnp.bfloat16, lo, hi)
    def permutation(self, n):
        return jax.random.permutation(self._next(), n)


kernel_name = 'sequential_preLN__spectral_gfnet__swiglu_ffn__prompt'

def _fwd_setup_inputs():
    _rng = _Rng(jax.random.key(int.from_bytes(__import__("os").urandom(4), "little")))
    _w = (lambda a: (lambda t: t.astype(jnp.bfloat16) if jnp.issubdtype(t.dtype, jnp.floating) else t)(jnp.asarray(a)))
    def _A_setup():
        B, S, D = 1, 2048, 576
        Df = D // 2 + 1
        return {
            "x": _w((lambda *s: _rng.normal(s) * 0.05)(B, S, D)),
            "w_r": _w((lambda *s: _rng.normal(s) * 0.05)(S, Df) * 0.02),
            "w_i": _w((lambda *s: _rng.normal(s) * 0.05)(S, Df) * 0.02),
        }
    _A_in = _A_setup()

    def _B_setup():
        B, S, D, F = 1, 2048, 576, 4608
        return {
            "x": _w((lambda *s: _rng.normal(s) * 0.05)(B, S, D)),
            "w_gate": _w((lambda *s: _rng.normal(s) * 0.05)(D, F)),
            "w_up": _w((lambda *s: _rng.normal(s) * 0.05)(D, F)),
            "w_down": _w((lambda *s: _rng.normal(s) * 0.05)(F, D)),
        }
    _B_in = _B_setup()

    return {
        "A_x": _A_in["x"],
        "A_w_r": _A_in["w_r"],
        "A_w_i": _A_in["w_i"],
        "B_x": _B_in["x"],
        "B_w_gate": _B_in["w_gate"],
        "B_w_up": _B_in["w_up"],
        "B_w_down": _B_in["w_down"],
    }

def _fwd_reference(A_x, A_w_r, A_w_i, B_x, B_w_gate, B_w_up, B_w_down):
    def _A_ref(x, w_r, w_i):
        B, S, D = x.shape
        X = (lambda x, axes=(-2,-1): jnp.fft.rfft2(x.astype(jnp.float32), axes=axes))(x, axes=(-2, -1))
        W = w_r + 1j * w_i
        X = X * W
        y = (lambda x, s, axes=(-2,-1): jnp.fft.irfft2(x, s=s, axes=axes).astype(jnp.bfloat16))(X, (S, D), axes=(-2, -1))
        return y

    def _B_ref(x, w_gate, w_up, w_down):
        g = _silu(x @ w_gate)
        u = x @ w_up
        return (g * u) @ w_down

    x = A_x
    h = x + _A_ref(_layernorm(x, axis=-1), A_w_r, A_w_i)
    h2 = h + _B_ref(_layernorm(h, axis=-1), B_w_gate, B_w_up, B_w_down)
    return h2


def setup_inputs():
    _inp = _fwd_setup_inputs()
    _gk = jax.random.fold_in(jax.random.key(int.from_bytes(__import__("os").urandom(4), "little")), 2**31 - 1)
    _shapes = [[1, 2048, 576]]
    _dtypes = ['bfloat16']
    _gks = jax.random.split(_gk, len(_shapes))
    _gs = [jax.random.normal(k, s, dtype=jnp.dtype(d)) * 0.05 for k, s, d in zip(_gks, _shapes, _dtypes)]
    _inp["grad_out"] = _gs[0]
    return _inp

def reference(A_x, A_w_r, A_w_i, B_w_gate, B_w_up, B_w_down, B_x, grad_out):
    _const = dict(B_x=B_x)
    def _f(*_d):
        return _fwd_reference(**{'A_x': _d[0], 'A_w_r': _d[1], 'A_w_i': _d[2], 'B_w_gate': _d[3], 'B_w_up': _d[4], 'B_w_down': _d[5], **_const})
    _out, _vjp = jax.vjp(_f, A_x, A_w_r, A_w_i, B_w_gate, B_w_up, B_w_down)
    _grads = _vjp(grad_out)
    _out0 = jnp.asarray(_out)
    return (_out0, *[jnp.asarray(_g) for _g in _grads])
```

```python
import numpy as np
import jax
import jax.numpy as jnp
from jax import lax
import jax.experimental.pallas as pl
import jax.experimental.pallas.tpu as pltpu

S, D, F = 2048, 576, 4608
DF = D // 2 + 1
DP = 384
H = S // 2
TF = 512
NF = F // TF
TM = 512
CH = 256
EPS = 1e-5
F32 = jnp.float32
BF16 = jnp.bfloat16

_NT = (((1,), (1,)), ((), ()))


def _dft_constants():
    k = np.arange(H, dtype=np.int64)
    s = np.arange(S, dtype=np.int64)
    r2 = np.zeros((S, S), np.float64)
    r2[:H] = np.cos(2 * np.pi * ((k[:, None] * s[None, :]) % S) / S)
    r2[H] = np.cos(np.pi * (s % 2))
    r2[H + 1:] = np.sin(2 * np.pi * ((k[1:, None] * s[None, :]) % S) / S)
    d = np.arange(D, dtype=np.int64)
    l = np.arange(DF, dtype=np.int64)
    fd = np.zeros((D, 2 * DP), np.float64)
    fd[:, :DF] = np.cos(2 * np.pi * ((d[:, None] * l[None, :]) % D) / D)
    fd[:, DP:DP + DF] = np.sin(2 * np.pi * ((d[:, None] * l[None, :]) % D) / D)
    cvt = lambda a: jnp.asarray(np.ascontiguousarray(a), dtype=BF16)
    return cvt(r2), cvt(r2.T), cvt(fd), cvt(fd.T)


def _dot(a, b):
    return jnp.dot(a, b, preferred_element_type=F32)


def _ln_stats(v):
    m = jnp.mean(v, axis=-1, keepdims=True)
    vc = v - m
    var = jnp.mean(vc * vc, axis=-1, keepdims=True)
    r = lax.rsqrt(var + EPS)
    return vc * r, r


def _ln_bwd(dy, xh, r):
    return r * (dy - jnp.mean(dy, axis=-1, keepdims=True)
                - xh * jnp.mean(dy * xh, axis=-1, keepdims=True))


def _kernel(x_ref, wr_ref, wi_ref, go_ref, wg_ref, wu_ref, wd_ref,
            r2_ref, r2t_ref, fd_ref, fdt_ref,
            h2_ref, dx_ref, dwr_ref, dwi_ref, dwg_ref, dwu_ref, dwd_ref,
            vbuf, eo, xf, wf, wpad, h_s, hn_s, hnT, goT, oacc, dacc,
            act_s, dgp_s, du_s):
    j = pl.program_id(0)

    def scale_vec():
        lane = lax.broadcasted_iota(jnp.int32, (1, DP), 1)
        c = jnp.where((lane == 0) | (lane == DF - 1), 1.0, 2.0)
        c = jnp.where(lane < DF, c, 0.0)
        return (c * (1.0 / (S * D))).astype(F32)

    def perm_matrix():
        r = lax.broadcasted_iota(jnp.int32, (H, H), 0)
        c = lax.broadcasted_iota(jnp.int32, (H, H), 1)
        return jnp.where(((r + c) & (H - 1)) == 0, 1.0, 0.0).astype(BF16)

    def spec_fwd(c):
        off = pl.multiple_of(c * CH, CH)
        v = vbuf[...]
        za = _dot(r2_ref[pl.ds(off, CH), :], v).astype(BF16)
        zb = _dot(r2_ref[pl.ds(H + off, CH), :], v).astype(BF16)
        p = _dot(za, fd_ref[...])
        q = _dot(zb, fd_ref[...])
        pc, ps = p[:, :DP], p[:, DP:]
        qc, qs = q[:, :DP], q[:, DP:]
        row0 = (lax.broadcasted_iota(jnp.int32, (CH, DP), 0) + off) == 0
        tr = jnp.where(row0, pc, pc - qs)
        ti = jnp.where(row0, -ps, -(ps + qc))
        br = jnp.where(row0, qc, pc + qs)
        bi = jnp.where(row0, -qs, qc - ps)
        return tr, ti, br, bi, row0

    def spec_inv_stage1(c, tr, ti, br, bi, row0):
        off = pl.multiple_of(c * CH, CH)
        e = jnp.concatenate([jnp.where(row0, tr, tr + br),
                             jnp.where(row0, -ti, -(ti + bi))], axis=1).astype(BF16)
        o = jnp.concatenate([jnp.where(row0, br, bi - ti),
                             jnp.where(row0, -bi, br - tr)], axis=1).astype(BF16)
        eo[pl.ds(off, CH), :] = _dot(e, fdt_ref[...]).astype(BF16)
        eo[pl.ds(H + off, CH), :] = _dot(o, fdt_ref[...]).astype(BF16)

    @pl.when(j == 0)
    def _prologue():
        def ln1(c, carry):
            rows = pl.ds(pl.multiple_of(c * CH, CH), CH)
            xh, _ = _ln_stats(x_ref[rows, :].astype(F32))
            vbuf[rows, :] = xh.astype(BF16)
            return carry
        lax.fori_loop(0, S // CH, ln1, 0)

        wpad[...] = jnp.zeros(wpad.shape, BF16)
        wpad[:, 0:DF] = wr_ref[...]
        wpad[:, DP:DP + DF] = wi_ref[...]
        wf[0:H, :] = wpad[0:H, :].astype(F32)
        wf[H:S, :] = _dot(perm_matrix(), wpad[H:S, :])

        sc = scale_vec()

        def fwd1(c, carry):
            off = pl.multiple_of(c * CH, CH)
            tr, ti, br, bi, row0 = spec_fwd(c)
            xf[pl.ds(off, CH), 0:DP] = tr
            xf[pl.ds(off, CH), DP:2 * DP] = ti
            xf[pl.ds(H + off, CH), 0:DP] = br
            xf[pl.ds(H + off, CH), DP:2 * DP] = bi
            wtr = wf[pl.ds(off, CH), 0:DP] * sc
            wti = wf[pl.ds(off, CH), DP:2 * DP] * sc
            wbr = wf[pl.ds(H + off, CH), 0:DP] * sc
            wbi = wf[pl.ds(H + off, CH), DP:2 * DP] * sc
            spec_inv_stage1(c, tr * wtr - ti * wti, tr * wti + ti * wtr,
                            br * wbr - bi * wbi, br * wbi + bi * wbr, row0)
            return carry
        lax.fori_loop(0, H // CH, fwd1, 0)

        def fwd2(c, carry):
            rows = pl.ds(pl.multiple_of(c * CH, CH), CH)
            y = _dot(r2t_ref[rows, :], eo[...]).astype(BF16)
            h = (x_ref[rows, :] + y).astype(F32)
            h_s[rows, :] = h
            oacc[rows, :] = h
            dacc[rows, :] = jnp.zeros((CH, D), F32)
            hh, _ = _ln_stats(h)
            hn_s[rows, :] = hh.astype(BF16)
            return carry
        lax.fori_loop(0, S // CH, fwd2, 0)

        hnT[...] = hn_s[...].astype(F32).T.astype(BF16)
        goT[...] = go_ref[...].astype(F32).T.astype(BF16)

    def chunk(c, carry):
        rows = pl.ds(pl.multiple_of(c * TM, TM), TM)
        hn = hn_s[rows, :]
        go = go_ref[rows, :]
        gp = _dot(hn, wg_ref[...])
        u = _dot(hn, wu_ref[...])
        da = lax.dot_general(go, wd_ref[...], _NT, preferred_element_type=F32)
        sg = 1.0 / (1.0 + jnp.exp(-gp))
        g = gp * sg
        act = (g * u).astype(BF16)
        dgp = (da * u * (sg * (1.0 + gp * (1.0 - sg)))).astype(BF16)
        du = (da * g).astype(BF16)
        act_s[rows, :] = act
        dgp_s[rows, :] = dgp
        du_s[rows, :] = du
        oacc[rows, :] += _dot(act, wd_ref[...])
        dacc[rows, :] += (
            lax.dot_general(dgp, wg_ref[...], _NT, preferred_element_type=F32)
            + lax.dot_general(du, wu_ref[...], _NT, preferred_element_type=F32))
        return carry
    lax.fori_loop(0, S // TM, chunk, 0)

    dwg_ref[...] = _dot(hnT[...], dgp_s[...]).astype(BF16)
    dwu_ref[...] = _dot(hnT[...], du_s[...]).astype(BF16)
    dwd_ref[...] = _dot(goT[...], act_s[...]).T.astype(BF16)

    @pl.when(j == NF - 1)
    def _epilogue():
        h2_ref[...] = oacc[...].astype(BF16)

        def bwd0(c, carry):
            rows = pl.ds(pl.multiple_of(c * CH, CH), CH)
            hh, r = _ln_stats(h_s[rows, :])
            dh = go_ref[rows, :].astype(F32) + _ln_bwd(dacc[rows, :], hh, r)
            dh = dh.astype(BF16)
            vbuf[rows, :] = dh
            return carry
        lax.fori_loop(0, S // CH, bwd0, 0)

        sc = scale_vec()

        def bwd1(c, carry):
            off = pl.multiple_of(c * CH, CH)
            tr, ti, br, bi, row0 = spec_fwd(c)
            tr, ti, br, bi = tr * sc, ti * sc, br * sc, bi * sc
            xtr = xf[pl.ds(off, CH), 0:DP]
            xti = xf[pl.ds(off, CH), DP:2 * DP]
            xbr = xf[pl.ds(H + off, CH), 0:DP]
            xbi = xf[pl.ds(H + off, CH), DP:2 * DP]
            wpad[pl.ds(off, CH), 0:DP] = (tr * xtr + ti * xti).astype(BF16)
            wpad[pl.ds(off, CH), DP:2 * DP] = (ti * xtr - tr * xti).astype(BF16)
            wpad[pl.ds(H + off, CH), 0:DP] = (br * xbr + bi * xbi).astype(BF16)
            wpad[pl.ds(H + off, CH), DP:2 * DP] = (bi * xbr - br * xbi).astype(BF16)
            wtr = wf[pl.ds(off, CH), 0:DP]
            wti = wf[pl.ds(off, CH), DP:2 * DP]
            wbr = wf[pl.ds(H + off, CH), 0:DP]
            wbi = wf[pl.ds(H + off, CH), DP:2 * DP]
            spec_inv_stage1(c, tr * wtr + ti * wti, ti * wtr - tr * wti,
                            br * wbr + bi * wbi, bi * wbr - br * wbi, row0)
            return carry
        lax.fori_loop(0, H // CH, bwd1, 0)

        def bwd2(c, carry):
            rows = pl.ds(pl.multiple_of(c * CH, CH), CH)
            gx = _dot(r2t_ref[rows, :], eo[...])
            xh, r = _ln_stats(x_ref[rows, :].astype(F32))
            dx = vbuf[rows, :].astype(F32) + _ln_bwd(gx, xh, r)
            dx_ref[rows, :] = dx.astype(BF16)
            return carry
        lax.fori_loop(0, S // CH, bwd2, 0)

        dwr_ref[0:H, :] = wpad[0:H, 0:DF]
        dwi_ref[0:H, :] = wpad[0:H, DP:DP + DF]
        bot = _dot(perm_matrix(), wpad[H:S, :]).astype(BF16)
        dwr_ref[H:S, :] = bot[:, 0:DF]
        dwi_ref[H:S, :] = bot[:, DP:DP + DF]


@jax.jit
def pallas_sequential_preLN__spectral_gfnet__swiglu_ffn__prompt_kernel(
    A_x: jax.Array,
    A_w_r: jax.Array,
    A_w_i: jax.Array,
    B_x: jax.Array,
    B_w_gate: jax.Array,
    B_w_up: jax.Array,
    B_w_down: jax.Array,
    grad_out: jax.Array,
):
    r2, r2t, fd, fdt = _dft_constants()
    x2 = A_x.reshape(S, D)
    go2 = grad_out.reshape(S, D)

    def full(shape):
        return pl.BlockSpec(shape, lambda j: (0, 0), pipeline_mode=pl.Buffered(1))

    in_specs = [
        full((S, D)), full((S, DF)), full((S, DF)), full((S, D)),
        pl.BlockSpec((D, TF), lambda j: (0, j)),
        pl.BlockSpec((D, TF), lambda j: (0, j)),
        pl.BlockSpec((TF, D), lambda j: (j, 0)),
        full((S, S)), full((S, S)), full((D, 2 * DP)), full((2 * DP, D)),
    ]
    out_specs = [
        pl.BlockSpec((S, D), lambda j: (0, 0)),
        pl.BlockSpec((S, D), lambda j: (0, 0)),
        pl.BlockSpec((S, DF), lambda j: (0, 0)),
        pl.BlockSpec((S, DF), lambda j: (0, 0)),
        pl.BlockSpec((D, TF), lambda j: (0, j)),
        pl.BlockSpec((D, TF), lambda j: (0, j)),
        pl.BlockSpec((TF, D), lambda j: (j, 0)),
    ]
    out_shape = [
        jax.ShapeDtypeStruct((S, D), BF16),
        jax.ShapeDtypeStruct((S, D), BF16),
        jax.ShapeDtypeStruct((S, DF), BF16),
        jax.ShapeDtypeStruct((S, DF), BF16),
        jax.ShapeDtypeStruct((D, F), BF16),
        jax.ShapeDtypeStruct((D, F), BF16),
        jax.ShapeDtypeStruct((F, D), BF16),
    ]
    scratch = [
        pltpu.VMEM((S, D), BF16),
        pltpu.VMEM((S, D), BF16),
        pltpu.VMEM((S, 2 * DP), F32),
        pltpu.VMEM((S, 2 * DP), F32),
        pltpu.VMEM((S, 2 * DP), BF16),
        pltpu.VMEM((S, D), F32),
        pltpu.VMEM((S, D), BF16),
        pltpu.VMEM((D, S), BF16),
        pltpu.VMEM((D, S), BF16),
        pltpu.VMEM((S, D), F32),
        pltpu.VMEM((S, D), F32),
        pltpu.VMEM((S, TF), BF16),
        pltpu.VMEM((S, TF), BF16),
        pltpu.VMEM((S, TF), BF16),
    ]
    h2, dx, dwr, dwi, dwg, dwu, dwd = pl.pallas_call(
        _kernel,
        grid=(NF,),
        in_specs=in_specs,
        out_specs=out_specs,
        out_shape=out_shape,
        scratch_shapes=scratch,
        compiler_params=pltpu.CompilerParams(
            dimension_semantics=("arbitrary",),
            vmem_limit_bytes=110 * 1024 * 1024,
        ),
    )(x2, A_w_r, A_w_i, go2, B_w_gate, B_w_up, B_w_down, r2, r2t, fd, fdt)
    return (h2.reshape(1, S, D), dx.reshape(1, S, D), dwr, dwi, dwg, dwu, dwd)
```

```python
import numpy as np
import jax
import jax.numpy as jnp
from jax import lax
import jax.experimental.pallas as pl
import jax.experimental.pallas.tpu as pltpu

S, D, F = 2048, 576, 4608
DF = D // 2 + 1
DP = 304
H = S // 2
Q = S // 4
TF = 512
NF = F // TF
TL = 512
TN = 256
CH = 128
EPS = 1e-5
F32 = jnp.float32
BF16 = jnp.bfloat16

_NT = (((1,), (1,)), ((), ()))


def _dft_constants():
    t = np.arange(Q, dtype=np.int64)
    a_ev = 2 * np.pi * ((t[:, None] * t[None, :]) % H) / H
    a_od = 2 * np.pi * ((t[:, None] * (2 * t[None, :] + 1)) % S) / S
    cee, see = np.cos(a_ev), np.sin(a_ev)
    ceo, seo = np.cos(a_od), np.sin(a_od)
    seo[0] = 1.0 - 2.0 * (t % 2)
    cf = np.concatenate([cee, ceo], axis=1)
    sf = np.concatenate([see, seo], axis=1)
    ti = np.concatenate([ceo.T, seo.T], axis=1)
    d = np.arange(D, dtype=np.int64)
    l = np.arange(DF, dtype=np.int64)
    fd = np.zeros((D, 2 * DP), np.float64)
    fd[:, :DF] = np.cos(2 * np.pi * ((d[:, None] * l[None, :]) % D) / D)
    fd[:, DP:DP + DF] = np.sin(2 * np.pi * ((d[:, None] * l[None, :]) % D) / D)
    cvt = lambda a: jnp.asarray(np.ascontiguousarray(a), dtype=BF16)
    return cvt(cf), cvt(sf), cvt(ti), cvt(fd), cvt(fd.T)


def _dot(a, b):
    return jnp.dot(a, b, preferred_element_type=F32)


def _dot_nt(a, b):
    return lax.dot_general(a, b, _NT, preferred_element_type=F32)


def _ln_stats_t(v):
    m = jnp.mean(v, axis=0, keepdims=True)
    vc = v - m
    var = jnp.mean(vc * vc, axis=0, keepdims=True)
    r = lax.rsqrt(var + EPS)
    return vc * r, r


def _ln_bwd_t(dy, xh, r):
    return r * (dy - jnp.mean(dy, axis=0, keepdims=True)
                - xh * jnp.mean(dy * xh, axis=0, keepdims=True))


def _sel(shape, cond_fn):
    r = lax.broadcasted_iota(jnp.int32, shape, 0)
    c = lax.broadcasted_iota(jnp.int32, shape, 1)
    return jnp.where(cond_fn(r, c), 1.0, 0.0).astype(BF16)


def _blk(ref, off, n=128):
    return ref[:, pl.ds(pl.multiple_of(off, 128), n)]


def _jrev():
    return _sel((256, 128), lambda r, c: r + c == 128)


def _tok_perm_block(src, dst, inverse, b):
    if inverse:
        lo = jnp.where(b < 4, Q + 128 * (3 - b), H + 128 * (7 - b))
        hi = lo + 128
        out = jnp.where(b < 4, 128 * (b + 4), 128 * (b + 8))
    else:
        lo = jnp.where(b < 4, 7 - b, 19 - b) * 128
        hi = jnp.where(b == 4, Q, lo + 128)
        out = Q + 128 * b
    blk = jnp.concatenate([_blk(src, lo), _blk(src, hi)], axis=1)
    dst[:, pl.ds(pl.multiple_of(out, 128), 128)] = _dot(blk, _jrev()).astype(dst.dtype)


def _tok_perm_rest(src, dst, inverse):
    isel = _sel((256, 128), lambda r, c: ((r == c) & (c > 0)) | ((r == 128) & (c == 0)))
    dst[:, 0:Q] = src[:, 0:Q]
    if inverse:
        dst[:, H + 128:H + Q] = src[:, 3 * Q + 128:S]
        blk = jnp.concatenate([src[:, 3 * Q:3 * Q + 128], src[:, Q:Q + 128]], axis=1)
        dst[:, H:H + 128] = _dot(blk, isel).astype(dst.dtype)
    else:
        dst[:, 3 * Q + 128:S] = src[:, H + 128:H + Q]
        blk = jnp.concatenate([src[:, H:H + 128], src[:, 3 * Q:3 * Q + 128]], axis=1)
        dst[:, 3 * Q:3 * Q + 128] = _dot(blk, isel).astype(dst.dtype)


def _tok_perm(src, dst, inverse):
    _tok_perm_rest(src, dst, inverse)

    def body(b, carry):
        _tok_perm_block(src, dst, inverse, b)
        return carry
    lax.fori_loop(0, 8, body, 0)


def _kernel(xT_hbm, wrT_hbm, wiT_hbm, goT_hbm, wg_hbm, wu_hbm, wdT_hbm,
            cf_hbm, sf_hbm, ti_hbm, fd_hbm, fdt_hbm,
            h2T_hbm, dxT_hbm, dwrT_hbm, dwiT_hbm, dwg_hbm, dwu_hbm, dwdT_hbm,
            xp, gop, ab, eoT, xf, wf, wpad, hT, hnT, oacc, dacc, alt, sp, rs,
            hn_s, go_s, act_s, dgp_s, du_s,
            xT_ref, wrT_ref, wiT_ref, goT_ref, cf_ref, sf_ref, ti_ref, fd_ref, fdt_ref,
            wbuf, obuf, sems, wsems, osems):
    j = pl.program_id(0)
    h2T_ref, dxT_ref, dwrT_ref, dwiT_ref = xT_ref, goT_ref, wrT_ref, wiT_ref
    slot = j % 2

    def w_copies(step, sl):
        cols = pl.ds(pl.multiple_of(step * TF, TF), TF)
        return [pltpu.make_async_copy(w.at[:, cols], wbuf.at[sl, i], wsems.at[sl, i])
                for i, w in enumerate((wg_hbm, wu_hbm, wdT_hbm))]

    def o_copies(step, sl):
        cols = pl.ds(pl.multiple_of(step * TF, TF), TF)
        return [pltpu.make_async_copy(obuf.at[sl, i], w.at[:, cols], osems.at[sl, i])
                for i, w in enumerate((dwg_hbm, dwu_hbm, dwdT_hbm))]

    wg_ref, wu_ref, wdT_ref = wbuf.at[slot, 0], wbuf.at[slot, 1], wbuf.at[slot, 2]
    dwg_ref, dwu_ref, dwdT_ref = obuf.at[slot, 0], obuf.at[slot, 1], obuf.at[slot, 2]

    in_copies = [pltpu.make_async_copy(src, dst, sems.at[i]) for i, (src, dst) in enumerate((
        (xT_hbm, xT_ref), (wrT_hbm, wrT_ref), (wiT_hbm, wiT_ref), (goT_hbm, goT_ref),
        (cf_hbm, cf_ref), (sf_hbm, sf_ref), (fdt_hbm, fdt_ref), (fd_hbm, fd_ref), (ti_hbm, ti_ref)))]
    out_copies = [pltpu.make_async_copy(src, dst, sems.at[9 + i]) for i, (src, dst) in enumerate((
        (h2T_ref, h2T_hbm), (dwrT_ref, dwrT_hbm), (dwiT_ref, dwiT_hbm),
        (dxT_ref.at[:, 0:Q], dxT_hbm.at[:, 0:Q]), (dxT_ref.at[:, H:H + Q], dxT_hbm.at[:, H:H + Q]),
        (dxT_ref.at[:, Q:H], dxT_hbm.at[:, Q:H]), (dxT_ref.at[:, H + Q:S], dxT_hbm.at[:, H + Q:S])))]

    def scale_vec():
        row = lax.broadcasted_iota(jnp.int32, (DP, 1), 0)
        c = jnp.where((row == 0) | (row == DF - 1), 1.0, 2.0)
        c = jnp.where(row < DF, c, 0.0)
        return (c * (1.0 / (S * D))).astype(F32)

    def sign_row():
        lane = lax.broadcasted_iota(jnp.int32, (1, CH), 1)
        return jnp.where((lane & 1) == 0, 1.0, -1.0).astype(F32)

    def quarters(c):
        off = pl.multiple_of(c * CH, CH)
        return [pl.ds(q * Q + off, CH) for q in range(4)]

    def fold_store(c, q0, q1, q2, q3):
        cols = quarters(c)
        col0 = (lax.broadcasted_iota(jnp.int32, (D, CH), 1) + c * CH) == 0
        s01, d01, s23, d23 = q0 + q1, q0 - q1, q2 + q3, q2 - q3
        aa = s01 + jnp.where(col0, 0.0, s23)
        ab[:, cols[0]] = aa.astype(BF16)
        ab[:, cols[1]] = (d01 + jnp.where(col0, 0.0, d23)).astype(BF16)
        ab[:, cols[2]] = (d01 - d23).astype(BF16)
        ab[:, cols[3]] = jnp.where(col0, d23, s01 - s23).astype(BF16)
        alt[...] += aa * sign_row()

        @pl.when(c == 0)
        def _():
            sp[...] = s23

    def special_cols():
        nyq = sp[:, 0:1]
        return nyq, jnp.sum(alt[...], axis=1, keepdims=True) + nyq

    def spec_fwd(c, v_mid, a_nyq):
        off = pl.multiple_of(c * CH, CH)
        qo = pl.multiple_of((c // 4) * Q, Q)
        col0d = (lax.broadcasted_iota(jnp.int32, (D, CH), 1) + off) == 0
        ev = jnp.where(c < 4, 1.0, 0.0).astype(F32)
        za = _dot(ab[:, pl.ds(qo, Q)], cf_ref[:, pl.ds(off, CH)]) + v_mid * (sign_row() * ev)
        zb = jnp.where(col0d, a_nyq, _dot(ab[:, pl.ds(H + qo, Q)], sf_ref[:, pl.ds(off, CH)]))
        p = _dot(fdt_ref[...], za.astype(BF16))
        q = _dot(fdt_ref[...], zb.astype(BF16))
        pc, ps = p[:DP], p[DP:]
        qc, qs = q[:DP], q[DP:]
        col0 = (lax.broadcasted_iota(jnp.int32, (DP, CH), 1) + off) == 0
        tr = jnp.where(col0, pc, pc - qs)
        ti = jnp.where(col0, -ps, -(ps + qc))
        br = jnp.where(col0, qc, pc + qs)
        bi = jnp.where(col0, -qs, qc - ps)
        return tr, ti, br, bi, col0

    def spec_inv_stage1(c, tr, ti, br, bi, col0):
        off = pl.multiple_of(c * CH, CH)
        ev = jnp.where(c < 4, 1.0, 0.0).astype(F32)
        e = jnp.concatenate([jnp.where(col0, tr, tr + br),
                             jnp.where(col0, -ti, -(ti + bi))], axis=0).astype(BF16)
        o = jnp.concatenate([jnp.where(col0, br, bi - ti),
                             jnp.where(col0, -bi, br - tr)], axis=0).astype(BF16)
        ee = _dot(fd_ref[...], e)
        oo = _dot(fd_ref[...], o)
        eoT[:, pl.ds(off, CH)] = ee.astype(BF16)
        eoT[:, pl.ds(H + off, CH)] = oo.astype(BF16)
        alt[...] += ee * (sign_row() * ev)

        @pl.when(c == 0)
        def _():
            sp[...] = oo

    def spec_inv_stage2(c, e_nyq, c_mid):
        off = pl.multiple_of(c * CH, CH)
        col0d = (lax.broadcasted_iota(jnp.int32, (D, CH), 1) + off) == 0
        cee = _dot(eoT[:, 0:Q], cf_ref[:, pl.ds(off, CH)]) + e_nyq * sign_row()
        ceo = _dot(eoT[:, Q:H], ti_ref[:, pl.ds(off, CH)])
        see = _dot(eoT[:, H:H + Q], sf_ref[:, pl.ds(off, CH)])
        seo = _dot(eoT[:, H + Q:S], ti_ref[:, pl.ds(Q + off, CH)])
        seo0 = jnp.where(col0d, 0.0, seo)
        p0, p1 = cee + ceo, cee - ceo
        m0, m1 = see + seo0, see - seo0
        return (p0 + m0, p1 - m1,
                jnp.where(col0d, c_mid + seo, p0 - m0),
                jnp.where(col0d, c_mid - seo, p1 + m1))

    @pl.when(j == 0)
    def _prologue():
        for cp in in_copies:
            cp.start()
        for cp in w_copies(0, 0):
            cp.start()
        in_copies[0].wait()
        with jax.named_scope("p_perm"):
            _tok_perm(xT_ref, xp, False)

        in_copies[1].wait()
        in_copies[2].wait()
        with jax.named_scope("p_ln1"):
            alt[...] = jnp.zeros(alt.shape, F32)
            wpad[...] = jnp.zeros(wpad.shape, BF16)
            wpad[0:DF, :] = wrT_ref[...]
            wpad[DP:DP + DF, :] = wiT_ref[...]

            def ln1(b, carry):
                vs = [_ln_stats_t(xp[:, cols].astype(F32))[0] for cols in quarters(b)]
                pe = _sel((256, 256), lambda r, c: ((c < 128) & (r == 2 * c)) | ((c >= 128) & (r == 2 * c - 255)))
                pr = _sel((384, 256), lambda r, c: ((c < 128) & (r == 256 - 2 * c)) | ((c >= 128) & (r == 511 - 2 * c)))
                o = pl.multiple_of(128 * b, 128)
                ev = _dot(_blk(wpad, 256 * b, 256), pe)
                wf[:, pl.ds(o, 128)] = ev[:, 0:128]
                wf[:, pl.ds(Q + o, 128)] = ev[:, 128:256]
                hi = jnp.where(b == 0, H, 256 * (8 - b))
                rv = _dot(jnp.concatenate([_blk(wpad, 256 * (7 - b), 256), _blk(wpad, hi)], axis=1), pr)
                wf[:, pl.ds(H + o, 128)] = rv[:, 0:128]
                wf[:, pl.ds(H + Q + o, 128)] = rv[:, 128:256]
                fold_store(b, *vs)
                return carry
            lax.fori_loop(0, Q // CH, ln1, 0)
            v_mid, a_nyq = special_cols()
            alt[...] = jnp.zeros(alt.shape, F32)

        for cp in in_copies[3:8]:
            cp.wait()
        sc = scale_vec()

        with jax.named_scope("p_fwd1"):
            _tok_perm_rest(goT_ref, gop, False)

            def fwd1(c, carry):
                off = pl.multiple_of(c * CH, CH)
                ct, cb = pl.ds(off, CH), pl.ds(H + off, CH)
                _tok_perm_block(goT_ref, gop, False, c)
                tr, ti, br, bi, col0 = spec_fwd(c, v_mid, a_nyq)
                xf[0:DP, ct] = tr
                xf[DP:2 * DP, ct] = ti
                xf[0:DP, cb] = br
                xf[DP:2 * DP, cb] = bi
                wtr = wf[0:DP, ct] * sc
                wti = wf[DP:2 * DP, ct] * sc
                wbr = wf[0:DP, cb] * sc
                wbi = wf[DP:2 * DP, cb] * sc
                spec_inv_stage1(c, tr * wtr - ti * wti, tr * wti + ti * wtr,
                                br * wbr - bi * wbi, br * wbi + bi * wbr, col0)
                return carry
            lax.fori_loop(0, H // CH, fwd1, 0)
            e_nyq, c_mid = special_cols()

        in_copies[8].wait()
        with jax.named_scope("p_fwd2"):
            def fwd2(c, carry):
                ys = spec_inv_stage2(c, e_nyq, c_mid)
                for y, cols in zip(ys, quarters(c)):
                    h = (xp[:, cols] + y.astype(BF16)).astype(F32)
                    oacc[:, cols] = h
                    dacc[:, cols] = jnp.zeros((D, CH), F32)
                    hh, r = _ln_stats_t(h)
                    hT[:, cols] = hh
                    rs[:, cols] = jnp.broadcast_to(r, (8, CH))
                    hnT[:, cols] = hh.astype(BF16)
                    hn_s[cols, :] = hh.T.astype(BF16)
                    go_s[cols, :] = gop[:, cols].astype(F32).T.astype(BF16)
                return carry
            lax.fori_loop(0, Q // CH, fwd2, 0)

    for cp in w_copies(j, slot):
        cp.wait()

    @pl.when(j + 1 < NF)
    def _():
        for cp in w_copies(j + 1, 1 - slot):
            cp.start()

    with jax.named_scope("ffn_chunks"):
        def chunk(c, carry):
            tok = pl.ds(pl.multiple_of(c * TL, TL), TL)
            hn = hn_s[tok, :]
            go = go_s[tok, :]
            gp = _dot(hn, wg_ref[...])
            u = _dot(hn, wu_ref[...])
            da = _dot(go, wdT_ref[...])
            sg = 1.0 / (1.0 + jnp.exp(-gp))
            g = gp * sg
            act = (g * u).astype(BF16)
            dgp = (da * u * (sg * (1.0 + gp * (1.0 - sg)))).astype(BF16)
            du = (da * g).astype(BF16)
            act_s[tok, :] = act
            dgp_s[tok, :] = dgp
            du_s[tok, :] = du
            oacc[:, tok] += _dot_nt(wdT_ref[...], act)
            dacc[:, tok] += _dot_nt(wg_ref[...], dgp) + _dot_nt(wu_ref[...], du)
            return carry
        lax.fori_loop(0, S // TL, chunk, 0)

    @pl.when(j >= 2)
    def _():
        for cp in o_copies(j - 2, slot):
            cp.wait()

    with jax.named_scope("ffn_dw"):
        def dwb(c, carry):
            cols = pl.ds(pl.multiple_of(c * TN, TN), TN)
            dwg_ref[:, cols] = _dot(hnT[...], dgp_s[:, cols]).astype(BF16)
            dwu_ref[:, cols] = _dot(hnT[...], du_s[:, cols]).astype(BF16)
            dwdT_ref[:, cols] = _dot(gop[...], act_s[:, cols]).astype(BF16)
            return carry
        lax.fori_loop(0, TF // TN, dwb, 0)
    for cp in o_copies(j, slot):
        cp.start()

    @pl.when(j == NF - 1)
    def _epilogue():
        with jax.named_scope("e_bwd0"):
            alt[...] = jnp.zeros(alt.shape, F32)

            def bwd0(c, carry):
                dhs = []
                for cols in quarters(c):
                    hnT[:, cols] = oacc[:, cols].astype(BF16)
                    dh = gop[:, cols].astype(F32) + _ln_bwd_t(dacc[:, cols], hT[:, cols], rs[0:1, cols])
                    dh = dh.astype(BF16).astype(F32)
                    oacc[:, cols] = dh
                    dhs.append(dh)
                fold_store(c, *dhs)
                return carry
            lax.fori_loop(0, Q // CH, bwd0, 0)
            v_mid, a_nyq = special_cols()
            alt[...] = jnp.zeros(alt.shape, F32)
            _tok_perm_rest(hnT, h2T_ref, True)

        sc = scale_vec()

        with jax.named_scope("e_bwd1"):
            def bwd1(c, carry):
                off = pl.multiple_of(c * CH, CH)
                ct, cb = pl.ds(off, CH), pl.ds(H + off, CH)
                _tok_perm_block(hnT, h2T_ref, True, c)
                tr, ti, br, bi, col0 = spec_fwd(c, v_mid, a_nyq)
                tr, ti, br, bi = tr * sc, ti * sc, br * sc, bi * sc
                xtr = xf[0:DP, ct]
                xti = xf[DP:2 * DP, ct]
                xbr = xf[0:DP, cb]
                xbi = xf[DP:2 * DP, cb]
                wpad[0:DP, ct] = (tr * xtr + ti * xti).astype(BF16)
                wpad[DP:2 * DP, ct] = (ti * xtr - tr * xti).astype(BF16)
                wpad[0:DP, cb] = (br * xbr + bi * xbi).astype(BF16)
                wpad[DP:2 * DP, cb] = (bi * xbr - br * xbi).astype(BF16)
                wtr = wf[0:DP, ct]
                wti = wf[DP:2 * DP, ct]
                wbr = wf[0:DP, cb]
                wbi = wf[DP:2 * DP, cb]
                spec_inv_stage1(c, tr * wtr + ti * wti, ti * wtr - tr * wti,
                                br * wbr + bi * wbi, bi * wbr - br * wbi, col0)
                return carry
            lax.fori_loop(0, H // CH, bwd1, 0)
            e_nyq, c_mid = special_cols()
            out_copies[0].start()

        with jax.named_scope("e_bwd2"):
            def bwd2(b, carry):
                pet = _sel((256, 256), lambda r, c: ((r < 128) & (c == 2 * r)) | ((r >= 128) & (c == 2 * r - 255)))
                pri = _sel((384, 256), lambda r, c: ((r < 128) & (2 * r + c == 256))
                           | ((r >= 128) & (r < 256) & (2 * r + c == 511)) | ((r == 256) & (c == 0)))
                lo = _dot(jnp.concatenate([_blk(wpad, 128 * b), _blk(wpad, Q + 128 * b)], axis=1),
                          pet).astype(BF16)
                o = pl.ds(pl.multiple_of(256 * b, 256), 256)
                dwrT_ref[:, o] = lo[0:DF]
                dwiT_ref[:, o] = lo[DP:DP + DF]
                hi = _dot(jnp.concatenate([_blk(wpad, H + 128 * (3 - b)), _blk(wpad, H + Q + 128 * (3 - b)),
                                           _blk(wpad, H + 128 * ((4 - b) & 3))], axis=1), pri).astype(BF16)
                o = pl.ds(pl.multiple_of(H + 256 * b, 256), 256)
                dwrT_ref[:, o] = hi[0:DF]
                dwiT_ref[:, o] = hi[DP:DP + DF]

                gs = spec_inv_stage2(b, e_nyq, c_mid)
                for gx, cols in zip(gs, quarters(b)):
                    xh, r = _ln_stats_t(xp[:, cols].astype(F32))
                    dx = oacc[:, cols] + _ln_bwd_t(gx, xh, r)
                    ab[:, cols] = dx.astype(BF16)
                return carry
            lax.fori_loop(0, Q // CH, bwd2, 0)
            out_copies[1].start()
            out_copies[2].start()
        with jax.named_scope("e_perm"):
            _tok_perm_rest(ab, dxT_ref, True)
            out_copies[3].start()
            out_copies[4].start()

            def pb(b, carry):
                _tok_perm_block(ab, dxT_ref, True, b)
                return carry
            lax.fori_loop(0, 4, pb, 0)
            out_copies[5].start()
            lax.fori_loop(4, 8, pb, 0)
            out_copies[6].start()
        for cp in out_copies:
            cp.wait()
        for cp in o_copies(j - 1, 1 - slot) + o_copies(j, slot):
            cp.wait()


@jax.jit
def pallas_sequential_preLN__spectral_gfnet__swiglu_ffn__prompt_kernel(
    A_x: jax.Array,
    A_w_r: jax.Array,
    A_w_i: jax.Array,
    B_x: jax.Array,
    B_w_gate: jax.Array,
    B_w_up: jax.Array,
    B_w_down: jax.Array,
    grad_out: jax.Array,
):
    cf, sf, ti, fd, fdt = _dft_constants()
    xT = A_x.reshape(S, D).T
    goT = grad_out.reshape(S, D).T

    hbm = pl.BlockSpec(memory_space=pl.ANY)
    in_specs = [hbm] * 12
    out_specs = [hbm] * 7
    out_shape = [
        jax.ShapeDtypeStruct((D, S), BF16),
        jax.ShapeDtypeStruct((D, S), BF16),
        jax.ShapeDtypeStruct((DF, S), BF16),
        jax.ShapeDtypeStruct((DF, S), BF16),
        jax.ShapeDtypeStruct((D, F), BF16),
        jax.ShapeDtypeStruct((D, F), BF16),
        jax.ShapeDtypeStruct((D, F), BF16),
    ]
    scratch = [
        pltpu.VMEM((D, S), BF16),
        pltpu.VMEM((D, S), BF16),
        pltpu.VMEM((D, S), BF16),
        pltpu.VMEM((D, S), BF16),
        pltpu.VMEM((2 * DP, S), F32),
        pltpu.VMEM((2 * DP, S), F32),
        pltpu.VMEM((2 * DP, S), BF16),
        pltpu.VMEM((D, S), F32),
        pltpu.VMEM((D, S), BF16),
        pltpu.VMEM((D, S), F32),
        pltpu.VMEM((D, S), F32),
        pltpu.VMEM((D, CH), F32),
        pltpu.VMEM((D, CH), F32),
        pltpu.VMEM((8, S), F32),
        pltpu.VMEM((S, D), BF16),
        pltpu.VMEM((S, D), BF16),
        pltpu.VMEM((S, TF), BF16),
        pltpu.VMEM((S, TF), BF16),
        pltpu.VMEM((S, TF), BF16),
        pltpu.VMEM((D, S), BF16),
        pltpu.VMEM((DF, S), BF16),
        pltpu.VMEM((DF, S), BF16),
        pltpu.VMEM((D, S), BF16),
        pltpu.VMEM((Q, H), BF16),
        pltpu.VMEM((Q, H), BF16),
        pltpu.VMEM((Q, H), BF16),
        pltpu.VMEM((D, 2 * DP), BF16),
        pltpu.VMEM((2 * DP, D), BF16),
        pltpu.VMEM((2, 3, D, TF), BF16),
        pltpu.VMEM((2, 3, D, TF), BF16),
        pltpu.SemaphoreType.DMA((16,)),
        pltpu.SemaphoreType.DMA((2, 3)),
        pltpu.SemaphoreType.DMA((2, 3)),
    ]
    h2T, dxT, dwrT, dwiT, dwg, dwu, dwdT = pl.pallas_call(
        _kernel,
        grid=(NF,),
        in_specs=in_specs,
        out_specs=out_specs,
        out_shape=out_shape,
        scratch_shapes=scratch,
        compiler_params=pltpu.CompilerParams(
            dimension_semantics=("arbitrary",),
            vmem_limit_bytes=110 * 1024 * 1024,
        ),
    )(xT, A_w_r.T, A_w_i.T, goT, B_w_gate, B_w_up, B_w_down.T, cf, sf, ti, fd, fdt)
    return (h2T.T.reshape(1, S, D), dxT.T.reshape(1, S, D), dwrT.T, dwiT.T,
            dwg, dwu, dwdT.T)
```
